```python
import os as _os
_os.environ.setdefault("JAX_PLATFORMS", "cpu")
import jax
import jax.numpy as jnp

def _softmax(x, axis=-1):
    return jax.nn.softmax(x, axis=axis)
def _gelu(x):
    return jax.nn.gelu(x, approximate=True)
def _silu(x):
    return jax.nn.silu(x)
def _sigmoid(x):
    return jax.nn.sigmoid(x)
def _layernorm(x, axis=-1, eps=1e-5):
    m = jnp.mean(x, axis=axis, keepdims=True)
    v = jnp.var(x, axis=axis, keepdims=True)
    return (x - m) / jnp.sqrt(v + eps)
def _scatter_add(tgt, idx, src, axis=0):
    return tgt.at[idx].add(src)
def _segment_sum(src, seg, n):
    return jax.ops.segment_sum(src, seg, n)
class _Rng:
    def __init__(self, key):
        self._k = key
    def _next(self):
        self._k, sub = jax.random.split(self._k)
        return sub
    def normal(self, shape):
        return jax.random.normal(self._next(), shape, dtype=jnp.bfloat16)
    def randint(self, lo, hi, shape):
        return jax.random.randint(self._next(), shape, lo, hi, dtype=jnp.int32)
    def uniform(self, shape, lo=0.0, hi=1.0):
        return jax.random.uniform(self._next(), shape, jnp.bfloat16, lo, hi)
    def permutation(self, n):
        return jax.random.permutation(self._next(), n)


kernel_name = 'sequential_preLN__linear_attn_block__glu_gated_reglu__prompt'

def setup_inputs():
    _rng = _Rng(jax.random.key(int.from_bytes(__import__("os").urandom(4), "little")))
    _w = (lambda a: (lambda t: t.astype(jnp.bfloat16) if jnp.issubdtype(t.dtype, jnp.floating) else t)(jnp.asarray(a)))
    def _A_setup():
        B, S, D = 1, 2048, 640
        return {
            "x": _w((lambda *s: _rng.normal(s) * 0.05)(B, S, D)),
            "wqkv": _w((lambda *s: _rng.normal(s) * 0.05)(D, 3 * D)),
            "wo": _w((lambda *s: _rng.normal(s) * 0.05)(D, D)),
        }
    _A_in = _A_setup()

    def _B_setup():
        B, S, D, F = 1, 2048, 640, 1536
        return {
            "x": _w((lambda *s: _rng.normal(s) * 0.05)(B, S, D)),
            "W_gate": _w((lambda *s: _rng.normal(s) * 0.05)(D, F) * (2.0 / D) ** 0.5),
            "W_up": _w((lambda *s: _rng.normal(s) * 0.05)(D, F) * (2.0 / D) ** 0.5),
            "W_down": _w((lambda *s: _rng.normal(s) * 0.05)(F, D) * (1.0 / F) ** 0.5),
        }
    _B_in = _B_setup()

    return {
        "A_x": _A_in["x"],
        "A_wqkv": _A_in["wqkv"],
        "A_wo": _A_in["wo"],
        "B_x": _B_in["x"],
        "B_W_gate": _B_in["W_gate"],
        "B_W_up": _B_in["W_up"],
        "B_W_down": _B_in["W_down"],
    }

def reference(A_x, A_wqkv, A_wo, B_x, B_W_gate, B_W_up, B_W_down):
    def _A_ref(x, wqkv, wo):
        B, S, D = x.shape
        H = 32; Dh = D // H
        qkv = (lambda x, *d: x.transpose(*d))((x @ wqkv).reshape(B, S, 3, H, Dh), 2, 0, 3, 1, 4)
        q, k, v = qkv[0], qkv[1], qkv[2]
        phi = lambda t: jnp.where(t > 0, t + 1, jnp.exp(t)) + 1e-6
        pq, pk = phi(q), phi(k)
        kv = jnp.einsum("bhsd,bhse->bhde", pk, v)
        z = jnp.einsum("bhsd->bhd", pk)
        num = jnp.einsum("bhqd,bhde->bhqe", pq, kv)
        den = jnp.einsum("bhqd,bhd->bhq", pq, z)[..., None] + 1e-6
        o = num / den
        return (lambda x, *d: x.transpose(*d))(o, 0, 2, 1, 3).reshape(B, S, D) @ wo

    def _B_ref(x, W_gate, W_up, W_down):
        gate = jnp.einsum("bsd,df->bsf", x, W_gate)
        up = jnp.einsum("bsd,df->bsf", x, W_up)
        gate = gate * (lambda x, dt: x.astype(dt))(gate > 0, gate.dtype)
        h = gate * up
        return jnp.einsum("bsf,fd->bsd", h, W_down)

    x = A_x
    h = x + _A_ref(_layernorm(x, axis=-1), A_wqkv, A_wo)
    h2 = h + _B_ref(_layernorm(h, axis=-1), B_W_gate, B_W_up, B_W_down)
    return h2
```

```python
import functools
import jax
import jax.numpy as jnp
from jax import lax
import jax.experimental.pallas as pl
import jax.experimental.pallas.tpu as pltpu

H = 32
T1 = 512
T3 = 512

def _ln(xf, d):
    m = jnp.sum(xf, axis=-1, keepdims=True) * (1.0 / d)
    c = xf - m
    v = jnp.sum(c * c, axis=-1, keepdims=True) * (1.0 / d)
    return c * lax.rsqrt(v + 1e-5)

def _phi(t):
    return jnp.where(t > 0, t + 1.0, jnp.exp(t)) + 1e-6

def _dot(a, b):
    return jnp.dot(a, b, preferred_element_type=jnp.float32)

def _kernel(x_hbm, wqkv_hbm, wo_hbm, wg_hbm, wu_hbm, wd_hbm, out_hbm,
            x_v, xn_v, wq_v, wk_v, wv_v, wo_v, wg_v, wu_v, wd_v, wkt_v,
            g_v, z_v, m_v, zc_v, e_v, out_v, sem_x, sem_w, sem_o):
    S, D = x_v.shape
    F = wg_v.shape[1]
    Dh = D // H
    n1 = S // T1
    n3 = S // T3

    def xcopy(i):
        return pltpu.make_async_copy(x_hbm.at[pl.ds(i * T1, T1)], x_v.at[pl.ds(i * T1, T1)], sem_x.at[i])
    def ocopy(i):
        return pltpu.make_async_copy(out_v.at[pl.ds(i * T3, T3)], out_hbm.at[pl.ds(i * T3, T3)], sem_o.at[i])
    cq = pltpu.make_async_copy(wqkv_hbm.at[:, pl.ds(0, D)], wq_v, sem_w.at[0])
    ck = pltpu.make_async_copy(wqkv_hbm.at[:, pl.ds(D, D)], wk_v, sem_w.at[1])
    cv = pltpu.make_async_copy(wqkv_hbm.at[:, pl.ds(2 * D, D)], wv_v, sem_w.at[2])
    co = pltpu.make_async_copy(wo_hbm, wo_v, sem_w.at[3])
    cg = pltpu.make_async_copy(wg_hbm, wg_v, sem_w.at[4])
    cu = pltpu.make_async_copy(wu_hbm, wu_v, sem_w.at[5])
    cd = pltpu.make_async_copy(wd_hbm, wd_v, sem_w.at[6])

    xcopy(0).start()
    ck.start()
    for i in range(1, n1):
        xcopy(i).start()
    cv.start(); co.start(); cq.start(); cg.start(); cu.start(); cd.start()

    ck.wait()
    wkt_v[...] = wk_v[...].T
    g_v[...] = jnp.zeros_like(g_v)
    z_v[...] = jnp.zeros_like(z_v)

    def p1(i, _):
        xcopy(i).wait()
        r = pl.ds(pl.multiple_of(i * T1, T1), T1)
        xn = _ln(x_v[r, :].astype(jnp.float32), D).astype(jnp.bfloat16)
        xn_v[r, :] = xn
        kt = lax.dot_general(wkt_v[...], xn, (((1,), (1,)), ((), ())), preferred_element_type=jnp.float32)
        pk = _phi(kt)
        zz = pk[:, 0:128]
        for j in range(1, T1 // 128):
            zz = zz + pk[:, j * 128:(j + 1) * 128]
        z_v[...] += zz
        g_v[...] += _dot(pk.astype(jnp.bfloat16), xn)
        return 0
    lax.fori_loop(0, n1, p1, 0)

    cv.wait(); co.wait()
    kv = _dot(g_v[...].astype(jnp.bfloat16), wv_v[...])
    ri = lax.broadcasted_iota(jnp.int32, (D, D), 0) // Dh
    ci = lax.broadcasted_iota(jnp.int32, (D, D), 1) // Dh
    kv = jnp.where(ri == ci, kv, 0.0).astype(jnp.bfloat16)
    m_v[...] = _dot(kv, wo_v[...]).astype(jnp.bfloat16)
    z = jnp.sum(z_v[...], axis=1, keepdims=True)
    ri2 = lax.broadcasted_iota(jnp.int32, (D, 128), 0) // Dh
    ci2 = lax.broadcasted_iota(jnp.int32, (D, 128), 1)
    zc_v[...] = jnp.where(ri2 == ci2, z, 0.0).astype(jnp.bfloat16)
    ri3 = lax.broadcasted_iota(jnp.int32, (128, D), 0)
    ci3 = lax.broadcasted_iota(jnp.int32, (128, D), 1) // Dh
    e_v[...] = jnp.where(ri3 == ci3, 1.0, 0.0).astype(jnp.bfloat16)
    cq.wait(); cg.wait(); cu.wait(); cd.wait()

    def p3(i, _):
        r = pl.ds(pl.multiple_of(i * T3, T3), T3)
        pq = _phi(_dot(xn_v[r, :], wq_v[...]))
        den = _dot(pq.astype(jnp.bfloat16), zc_v[...]) + 1e-6
        lane = lax.broadcasted_iota(jnp.int32, den.shape, 1)
        rec = jnp.where(lane < H, 1.0 / den, 0.0).astype(jnp.bfloat16)
        rexp = _dot(rec, e_v[...])
        pqs = (pq * rexp).astype(jnp.bfloat16)
        h = x_v[r, :].astype(jnp.float32) + _dot(pqs, m_v[...])
        hn = _ln(h, D).astype(jnp.bfloat16)
        g = _dot(hn, wg_v[...])
        u = _dot(hn, wu_v[...])
        a = (jnp.maximum(g, 0.0) * u).astype(jnp.bfloat16)
        y = _dot(a, wd_v[...])
        out_v[r, :] = (h + y).astype(jnp.bfloat16)
        ocopy(i).start()
        return 0
    lax.fori_loop(0, n3, p3, 0)
    for i in range(n3):
        ocopy(i).wait()


@jax.jit
def pallas_sequential_preLN__linear_attn_block__glu_gated_reglu__prompt_kernel(
    A_x, A_wqkv, A_wo, B_x, B_W_gate, B_W_up, B_W_down):
    B, S, D = A_x.shape
    F = B_W_gate.shape[1]
    x2 = A_x.reshape(B * S, D)
    bf = jnp.bfloat16
    any_spec = pl.BlockSpec(memory_space=pl.ANY)
    out = pl.pallas_call(
        _kernel,
        out_shape=jax.ShapeDtypeStruct((B * S, D), A_x.dtype),
        in_specs=[any_spec] * 6,
        out_specs=any_spec,
        scratch_shapes=[
            pltpu.VMEM((S, D), bf), pltpu.VMEM((S, D), bf),
            pltpu.VMEM((D, D), bf), pltpu.VMEM((D, D), bf), pltpu.VMEM((D, D), bf), pltpu.VMEM((D, D), bf),
            pltpu.VMEM((D, F), bf), pltpu.VMEM((D, F), bf), pltpu.VMEM((F, D), bf),
            pltpu.VMEM((D, D), bf),
            pltpu.VMEM((D, D), jnp.float32), pltpu.VMEM((D, 128), jnp.float32),
            pltpu.VMEM((D, D), bf), pltpu.VMEM((D, 128), bf), pltpu.VMEM((128, D), bf),
            pltpu.VMEM((S, D), bf),
            pltpu.SemaphoreType.DMA((S // T1,)), pltpu.SemaphoreType.DMA((7,)), pltpu.SemaphoreType.DMA((S // T3,)),
        ],
        compiler_params=pltpu.CompilerParams(vmem_limit_bytes=100 * 1024 * 1024),
    )(x2, A_wqkv, A_wo, B_W_gate, B_W_up, B_W_down)
    return out.reshape(B, S, D)
```

```python
import jax
import jax.numpy as jnp
from jax import lax
import jax.experimental.pallas as pl
import jax.experimental.pallas.tpu as pltpu

H = 32
T1 = 512
T3 = 512
NSPLIT = 4
LNC = 64
BANDS = ((0, 144), (112, 272), (240, 400), (368, 528), (496, 640))
SCHED = "q0 q1 d0 q2 d1 a0 q3 d2 a1 d3 a2 g0 a3 g1 y0 g2 y1 g3 y2 y3"


def _ln(xf, d):
    m = jnp.sum(xf, axis=-1, keepdims=True) * (1.0 / d)
    c = xf - m
    v = jnp.sum(c * c, axis=-1, keepdims=True) * (1.0 / d)
    return c * lax.rsqrt(v + 1e-5)


def _phi(t):
    return jnp.where(t > 0, t + 1.0, jnp.exp(t)) + 1e-6


def _dot(a, b):
    return jnp.dot(a, b, preferred_element_type=jnp.float32)


def _head(idx):
    return lax.shift_right_logical(idx * 3277, 16)


def _kernel(x_hbm, wqkv_hbm, wo_hbm, wg_hbm, wu_hbm, wd_hbm, out_hbm,
            x_v, xn_v, wq_v, wk_v, wv_v, wo_v, wg_v, wu_v, wd_v,
            g_v, z_v, m_v, zc_v, out_v, sem_x, sem_w, sem_o):
    S, D = x_v.shape
    n1 = S // T1
    n3 = S // T3
    hs = T3 // NSPLIT
    f32, bf16 = jnp.float32, jnp.bfloat16

    def xcopy(i):
        return pltpu.make_async_copy(
            x_hbm.at[pl.ds(i * T1, T1)], x_v.at[pl.ds(i * T1, T1)], sem_x.at[i])

    def ocopy(i):
        return pltpu.make_async_copy(
            out_v.at[pl.ds(i * hs, hs)], out_hbm.at[pl.ds(i * hs, hs)], sem_o.at[i])

    cq = pltpu.make_async_copy(wqkv_hbm.at[:, pl.ds(0, D)], wq_v, sem_w.at[0])
    ck = pltpu.make_async_copy(wqkv_hbm.at[:, pl.ds(D, D)], wk_v, sem_w.at[1])
    cv = pltpu.make_async_copy(wqkv_hbm.at[:, pl.ds(2 * D, D)], wv_v, sem_w.at[2])
    co = pltpu.make_async_copy(wo_hbm, wo_v, sem_w.at[3])
    cg = pltpu.make_async_copy(wg_hbm, wg_v, sem_w.at[4])
    cu = pltpu.make_async_copy(wu_hbm, wu_v, sem_w.at[5])
    cd = pltpu.make_async_copy(wd_hbm, wd_v, sem_w.at[6])

    def ln_tile(start):
        for c in range(0, T1, LNC):
            rc = pl.ds(pl.multiple_of(start + c, LNC), LNC)
            xn_v[rc, :] = _ln(x_v[rc, :].astype(f32), D).astype(bf16)

    xcopy(0).start()
    ck.start()
    g_v[...] = jnp.zeros_like(g_v)
    z_v[...] = jnp.zeros_like(z_v)
    xcopy(0).wait()
    xcopy(1).start()
    ln_tile(jnp.int32(0))
    ck.wait()
    for i in range(2, n1):
        xcopy(i).start()
    cv.start()
    co.start()

    def p1(i, _):
        @pl.when(i + 1 < n1)
        def _():
            xcopy(i + 1).wait()

        @pl.when(i == 1)
        def _():
            cq.start()
            cg.start()
            cu.start()
            cd.start()

        xn = xn_v[pl.ds(pl.multiple_of(i * T1, T1), T1), :]
        pk = _phi(_dot(xn, wk_v[...]))
        ln_tile(jnp.minimum(i + 1, n1 - 1) * T1)
        z_v[...] += jnp.sum(pk.reshape(T1 // 8, 8, D), axis=0)
        g_v[...] += lax.dot_general(
            pk.astype(bf16), xn, (((0,), (0,)), ((), ())), preferred_element_type=f32)
        return 0

    lax.fori_loop(0, n1, p1, 0)

    cv.wait()
    co.wait()
    ms = []
    for j, (r0, r1) in enumerate(BANDS):
        kv = _dot(g_v[r0:r1, :].astype(bf16), wv_v[:, j * 128:(j + 1) * 128])
        ri = _head(lax.broadcasted_iota(jnp.int32, kv.shape, 0) + r0)
        ci = _head(lax.broadcasted_iota(jnp.int32, kv.shape, 1) + j * 128)
        kv = jnp.where(ri == ci, kv, 0.0).astype(bf16)
        ms.append(_dot(kv, wo_v[j * 128:(j + 1) * 128, :]))
    for j, (r0, r1) in enumerate(BANDS):
        lo = r0 if j == 0 else BANDS[j - 1][1]
        hi = r1 if j == len(BANDS) - 1 else BANDS[j + 1][0]
        m_v[lo:hi, :] = ms[j][lo - r0:hi - r0, :].astype(bf16)
        if j + 1 < len(BANDS):
            m_v[hi:r1, :] = (ms[j][hi - r0:, :] + ms[j + 1][:r1 - hi, :]).astype(bf16)
    z = jnp.sum(z_v[...], axis=0, keepdims=True)
    rh = lax.broadcasted_iota(jnp.int32, (H, D), 0)
    ch = _head(lax.broadcasted_iota(jnp.int32, (H, D), 1))
    zc_v[...] = jnp.where(rh == ch, z, 0.0).astype(bf16)
    cq.wait()
    cg.wait()
    cu.wait()
    cd.wait()

    def p3(i, _):
        rs = [pl.ds(pl.multiple_of(i * T3 + s * hs, hs), hs) for s in range(NSPLIT)]
        val = {}

        def st_den(p):
            dt = lax.dot_general(zc_v[...], p.astype(bf16), (((1,), (1,)), ((), ())),
                                 preferred_element_type=f32) + 1e-6
            rec = jnp.concatenate([1.0 / dt, jnp.ones((128 - H, hs), f32)], axis=0).T
            lane = lax.broadcasted_iota(jnp.int32, rec.shape, 1)
            rexp = jnp.concatenate(
                [jnp.take_along_axis(rec, _head(lane + j * 128), axis=1,
                                     mode="promise_in_bounds")
                 for j in range(D // 128)], axis=1)
            return (p * rexp).astype(bf16)

        for tok in SCHED.split():
            st, c = tok[0], int(tok[1])
            if st == "q":
                val["q", c] = _phi(_dot(xn_v[rs[c], :], wq_v[...]))
            elif st == "d":
                val["d", c] = st_den(val["q", c])
            elif st == "a":
                h = x_v[rs[c], :].astype(f32) + _dot(val["d", c], m_v[...])
                val["a", c] = (h, _ln(h, D).astype(bf16))
            elif st == "g":
                hn = val["a", c][1]
                g = _dot(hn, wg_v[...])
                u = _dot(hn, wu_v[...])
                val["g", c] = (jnp.maximum(g, 0.0) * u).astype(bf16)
            else:
                y = _dot(val["g", c], wd_v[...])
                out_v[rs[c], :] = (val["a", c][0] + y).astype(bf16)
                ocopy(i * NSPLIT + c).start()
        return 0

    lax.fori_loop(0, n3, p3, 0)
    for i in range(n3 * NSPLIT):
        ocopy(i).wait()


@jax.jit
def pallas_sequential_preLN__linear_attn_block__glu_gated_reglu__prompt_kernel(
    A_x: jax.Array,
    A_wqkv: jax.Array,
    A_wo: jax.Array,
    B_x: jax.Array,
    B_W_gate: jax.Array,
    B_W_up: jax.Array,
    B_W_down: jax.Array,
):
    B, S, D = A_x.shape
    F = B_W_gate.shape[1]
    bf, f32 = jnp.bfloat16, jnp.float32
    any_spec = pl.BlockSpec(memory_space=pl.ANY)
    out = pl.pallas_call(
        _kernel,
        out_shape=jax.ShapeDtypeStruct((B * S, D), A_x.dtype),
        in_specs=[any_spec] * 6,
        out_specs=any_spec,
        scratch_shapes=[
            pltpu.VMEM((S, D), bf), pltpu.VMEM((S, D), bf),
            pltpu.VMEM((D, D), bf), pltpu.VMEM((D, D), bf),
            pltpu.VMEM((D, D), bf), pltpu.VMEM((D, D), bf),
            pltpu.VMEM((D, F), bf), pltpu.VMEM((D, F), bf), pltpu.VMEM((F, D), bf),
            pltpu.VMEM((D, D), f32), pltpu.VMEM((8, D), f32),
            pltpu.VMEM((D, D), bf), pltpu.VMEM((H, D), bf),
            pltpu.VMEM((S, D), bf),
            pltpu.SemaphoreType.DMA((S // T1,)),
            pltpu.SemaphoreType.DMA((7,)),
            pltpu.SemaphoreType.DMA((S // T3 * NSPLIT,)),
        ],
        compiler_params=pltpu.CompilerParams(
            vmem_limit_bytes=100 * 1024 * 1024,
            flags={"XLA_TPU_EVENLY_DISTRIBUTE_CRITICAL_NODES": True},
            disable_semaphore_checks=True,
        ),
    )(A_x.reshape(B * S, D), A_wqkv, A_wo, B_W_gate, B_W_up, B_W_down)
    return out.reshape(B, S, D)
```
